```python
import jax
import jax.numpy as jnp

def _softmax(x, axis=-1):
    return jax.nn.softmax(x, axis=axis)
def _gelu(x):
    return jax.nn.gelu(x, approximate=True)
def _silu(x):
    return jax.nn.silu(x)
def _sigmoid(x):
    return jax.nn.sigmoid(x)
def _layernorm(x, axis=-1, eps=1e-5):
    m = jnp.mean(x, axis=axis, keepdims=True)
    v = jnp.var(x, axis=axis, keepdims=True)
    return (x - m) / jnp.sqrt(v + eps)
def _scatter_add(tgt, idx, src, axis=0):
    return tgt.at[idx].add(src)
def _segment_sum(src, seg, n):
    return jax.ops.segment_sum(src, seg, n)
class _Rng:
    def __init__(self, key):
        self._k = key
    def _next(self):
        self._k, sub = jax.random.split(self._k)
        return sub
    def normal(self, shape):
        return jax.random.normal(self._next(), shape, dtype=jnp.bfloat16)
    def randint(self, lo, hi, shape):
        return jax.random.randint(self._next(), shape, lo, hi, dtype=jnp.int32)
    def uniform(self, shape, lo=0.0, hi=1.0):
        return jax.random.uniform(self._next(), shape, jnp.bfloat16, lo, hi)
    def permutation(self, n):
        return jax.random.permutation(self._next(), n)


kernel_name = 'concat_heads__gqa_block_cached__mha_block_cached__near_ridge'

def setup_inputs():
    _rng = _Rng(jax.random.key(int.from_bytes(__import__("os").urandom(4), "little")))
    _w = (lambda a: (lambda t: t.astype(jnp.bfloat16) if jnp.issubdtype(t.dtype, jnp.floating) else t)(jnp.asarray(a)))
    def _A_setup():
        B, Sq, D = 16, 160, 640
        Hq, Hkv, Sk, Dh = 32, 32, 512, 192
        assert Hq % Hkv == 0, (Hq, Hkv)
        return {
            "x": _w((lambda *s: _rng.normal(s) * 0.05)(B, Sq, D)),
            "k_cache": _w((lambda *s: _rng.normal(s) * 0.05)(B, Hkv, Sk, Dh)),
            "v_cache": _w((lambda *s: _rng.normal(s) * 0.05)(B, Hkv, Sk, Dh)),
            "wq": _w((lambda *s: _rng.normal(s) * 0.05)(D, Hq * Dh) * (D ** -0.5)),
            "wo": _w((lambda *s: _rng.normal(s) * 0.05)(Hq * Dh, D) * ((Hq * Dh) ** -0.5)),
        }
    _A_in = _A_setup()

    def _B_setup():
        B, Sq, D = 16, 160, 640
        H, Sk, Dh = 32, 512, 192
        return {
            "x": _w((lambda *s: _rng.normal(s) * 0.05)(B, Sq, D)),
            "k_cache": _w((lambda *s: _rng.normal(s) * 0.05)(B, H, Sk, Dh)),
            "v_cache": _w((lambda *s: _rng.normal(s) * 0.05)(B, H, Sk, Dh)),
            "wq": _w((lambda *s: _rng.normal(s) * 0.05)(D, H * Dh) * (D ** -0.5)),
            "wo": _w((lambda *s: _rng.normal(s) * 0.05)(H * Dh, D) * ((H * Dh) ** -0.5)),
        }
    _B_in = _B_setup()

    return {
        "A_x": _A_in["x"],
        "A_k_cache": _A_in["k_cache"],
        "A_v_cache": _A_in["v_cache"],
        "A_wq": _A_in["wq"],
        "A_wo": _A_in["wo"],
        "B_x": _B_in["x"],
        "B_k_cache": _B_in["k_cache"],
        "B_v_cache": _B_in["v_cache"],
        "B_wq": _B_in["wq"],
        "B_wo": _B_in["wo"],
    }

def reference(A_x, A_k_cache, A_v_cache, A_wq, A_wo, B_x, B_k_cache, B_v_cache, B_wq, B_wo):
    def _A_ref(x, k_cache, v_cache, wq, wo):
        B, Sq, D = x.shape
        Hq, Dh = 32, 192
        Hkv = k_cache.shape[1]
        rep = Hq // Hkv
        q = (lambda x, *d: x.transpose(*d))((x @ wq).reshape(B, Sq, Hq, Dh), 0, 2, 1, 3)
        k = jnp.repeat(k_cache, rep, axis=1)
        v = jnp.repeat(v_cache, rep, axis=1)
        scores = jnp.einsum("bhqd,bhkd->bhqk", q, k) * (Dh ** -0.5)
        p = _softmax(scores, axis=-1)
        o = jnp.einsum("bhqk,bhkd->bhqd", p, v)
        return (lambda x, *d: x.transpose(*d))(o, 0, 2, 1, 3).reshape(B, Sq, Hq * Dh) @ wo

    def _B_ref(x, k_cache, v_cache, wq, wo):
        B, Sq, D = x.shape
        H, Dh = 32, 192
        q = (lambda x, *d: x.transpose(*d))((x @ wq).reshape(B, Sq, H, Dh), 0, 2, 1, 3)
        scores = jnp.einsum("bhqd,bhkd->bhqk", q, k_cache) * (Dh ** -0.5)
        p = _softmax(scores, axis=-1)
        o = jnp.einsum("bhqk,bhkd->bhqd", p, v_cache)
        return (lambda x, *d: x.transpose(*d))(o, 0, 2, 1, 3).reshape(B, Sq, H * Dh) @ wo

    a = _A_ref(A_x, A_k_cache, A_v_cache, A_wq, A_wo)
    b = _B_ref(B_x, B_k_cache, B_v_cache, B_wq, B_wo)
    return jnp.concatenate([a, b], axis=-1)
```

```python
import functools
import jax
import jax.numpy as jnp
from jax import lax
import jax.experimental.pallas as pl
import jax.experimental.pallas.tpu as pltpu

B, SQ, D, H, SK, DH = 16, 160, 640, 32, 512, 192
PAIR = 2 * DH
LOG2E = 1.4426950408889634

NT = (((1,), (1,)), ((), ()))


def _pair_attn(q, kt_ref, vt_ref, r0):
    c = (DH ** -0.5) * LOG2E
    lane = lax.broadcasted_iota(jnp.int32, (SQ, 128), 1)
    lo = lane < 64
    q0, q1, q2 = q[:, 0:128], q[:, 128:256], q[:, 256:384]
    z = jnp.zeros_like(q1)
    qa = jnp.concatenate([q0, jnp.where(lo, q1, z)], axis=1)
    qb = jnp.concatenate([jnp.where(lo, z, q1), q2], axis=1)
    outs = []
    for j, qq in enumerate((qa, qb)):
        kk = kt_ref[pl.ds(r0 + 128 * j, 256), :]
        s = jnp.dot(qq, kk, preferred_element_type=jnp.float32)
        m = jnp.max(s, axis=1, keepdims=True)
        p = jnp.exp2((s - m) * c)
        l = jnp.sum(p, axis=1, keepdims=True)
        vv = vt_ref[pl.ds(r0 + 128 * j, 256), :]
        o = lax.dot_general(p.astype(jnp.bfloat16), vv, NT, preferred_element_type=jnp.float32)
        outs.append(o * (1.0 / l))
    oa, ob = outs
    o = jnp.concatenate([oa[:, :128], jnp.where(lo, oa[:, 128:], ob[:, :128]), ob[:, 128:]], axis=1)
    return o.astype(jnp.bfloat16)


def build(A_x, A_k, A_v, A_wq, A_wo, B_x, B_k, B_v, B_wq, B_wo, G=4):
    W = G * PAIR
    NG = H * DH // W

    def tr(a):
        return jnp.transpose(a, (0, 1, 3, 2)).reshape(B, H * DH, SK)

    def kernel(ax, ak, av, awq, awo, bx, bk, bv, bwq, bwo, out, acc):
        g = pl.program_id(1)
        col = pl.multiple_of(g * W, 128)
        res = []
        for (x, k, v, wq, wo) in ((ax, ak, av, awq, awo), (bx, bk, bv, bwq, bwo)):
            q = jnp.dot(x[...], wq[:, pl.ds(col, W)], preferred_element_type=jnp.float32).astype(jnp.bfloat16)
            os_ = [_pair_attn(q[:, i * PAIR:(i + 1) * PAIR], k, v, i * PAIR) for i in range(G)]
            o = jnp.concatenate(os_, axis=1) if G > 1 else os_[0]
            res.append(jnp.dot(o, wo[pl.ds(col, W), :], preferred_element_type=jnp.float32))
        r = jnp.concatenate(res, axis=1)

        @pl.when(g == 0)
        def _():
            acc[...] = r

        @pl.when(g > 0)
        def _():
            acc[...] += r

        @pl.when(g == NG - 1)
        def _():
            out[...] = acc[...].astype(out.dtype)

    xs = pl.BlockSpec((None, SQ, D), lambda b, g: (b, 0, 0))
    ks = pl.BlockSpec((None, W, SK), lambda b, g: (b, g, 0))
    wqs = pl.BlockSpec((D, H * DH), lambda b, g: (0, 0), pipeline_mode=pl.Buffered(1))
    wos = pl.BlockSpec((H * DH, D), lambda b, g: (0, 0), pipeline_mode=pl.Buffered(1))
    return pl.pallas_call(
        kernel,
        grid=(B, NG),
        in_specs=[xs, ks, ks, wqs, wos] * 2,
        out_specs=pl.BlockSpec((None, SQ, 2 * D), lambda b, g: (b, 0, 0)),
        out_shape=jax.ShapeDtypeStruct((B, SQ, 2 * D), jnp.bfloat16),
        scratch_shapes=[pltpu.VMEM((SQ, 2 * D), jnp.float32)],
        compiler_params=pltpu.CompilerParams(
            dimension_semantics=("arbitrary", "arbitrary"),
            vmem_limit_bytes=100 * 1024 * 1024),
    )(A_x, tr(A_k), tr(A_v), A_wq, A_wo, B_x, tr(B_k), tr(B_v), B_wq, B_wo)


@jax.jit
def pallas_concat_heads__gqa_block_cached__mha_block_cached__near_ridge_kernel(
        A_x, A_k_cache, A_v_cache, A_wq, A_wo, B_x, B_k_cache, B_v_cache, B_wq, B_wo):
    return build(A_x, A_k_cache, A_v_cache, A_wq, A_wo, B_x, B_k_cache, B_v_cache, B_wq, B_wo)
```

```python
import functools, contextlib
import jax
import jax.numpy as jnp
from jax import lax
import jax.experimental.pallas as pl
import jax.experimental.pallas.tpu as pltpu

B, SQ, D, H, SK, DH = 16, 160, 640, 32, 512, 192
PAIR = 2 * DH
LOG2E = 1.4426950408889634
NT = (((1,), (1,)), ((), ()))
f32, bf16 = jnp.float32, jnp.bfloat16
HQ = SQ // 2


def dot(a, b):
    return jnp.dot(a, b, preferred_element_type=f32)


def dot_nt(a, b):
    return lax.dot_general(a, b, NT, preferred_element_type=f32)


def go(cp, op):
    return cp.start() if op == 'start' else cp.wait()


def build(A_x, A_k, A_v, A_wq, A_wo, B_x, B_k, B_v, B_wq, B_wo, NB=4, R=12, sched=None, norm=True,
          pat="Q2-A1-V0-B1-O9", nobc=False, flags=None, NPX=None, scopes=False, UP=1, only=None):
    NP = NPX or H // 2
    NT_ = NP * B
    c = (DH ** -0.5) * LOG2E
    pat = [(p[0], int(p[1]) if int(p[1]) < 5 else int(p[1]) - 10) for p in pat.split("-")]

    def tr(a):
        return jnp.transpose(a, (0, 1, 3, 2)).reshape(B, H * DH, SK)

    def kernel(ax, ak, av, awq, awo, bx, bk, bv, bwq, bwo, out,
               xbuf, kbuf, vbuf, wqbuf, wobuf, acc, obuf, cbuf, xsem, kvsem, wqsem, wosem, osem):
        X, KV, WQ, WO = (ax, bx), ((ak, bk), (av, bv)), (awq, bwq), (awo, bwo)
        kvbuf = (kbuf, vbuf)
        four = [(w, s) for w in range(2) for s in range(2)]

        def rows(g):
            return pl.ds(g * PAIR if isinstance(g, int) else pl.multiple_of(g * PAIR, 128), PAIR)

        def x_cp(b, s):
            return pltpu.make_async_copy(X[s].at[b], xbuf.at[s, b], xsem.at[s, b])

        def kv_cp(t, n, w, s):
            return pltpu.make_async_copy(KV[w][s].at[pl.ds(t % B, n), rows(t // B)],
                                         kvbuf[w].at[s, pl.ds(t % R, n)], kvsem.at[t % R, w, s])

        def wq_cp(g, s):
            return pltpu.make_async_copy(WQ[s].at[:, rows(g)], wqbuf.at[g % 2, s], wqsem.at[g % 2, s])

        def wo_cp(g, s):
            return pltpu.make_async_copy(WO[s].at[rows(g)], wobuf.at[g % 2, s], wosem.at[g % 2, s])

        def o_cp(b):
            return pltpu.make_async_copy(obuf.at[b], out.at[b], osem.at[b])

        def lo_mask(n):
            return lax.broadcasted_iota(jnp.int32, (n, 128), 1) < 64

        def compute(g, b0, nb, first=False, last=False):
            t = g * B + b0
            r0 = t % R
            ws = g % 2
            units = [(s, i) for i in range(nb) for s in range(2)]
            U = len(units)
            st = [dict() for _ in units]

            def Qp(u):
                s, i = units[u]
                q = dot(xbuf[s, b0 + i], wqbuf[ws, s])
                lo = lo_mask(HQ)
                rnd = lambda z: z.astype(bf16).astype(f32)
                t0, t1, t2 = q[:HQ, 0:128], rnd(q[:HQ, 128:256]), q[:HQ, 256:384]
                b0_, b1, b2 = rnd(q[HQ:, 0:128]), q[HQ:, 128:256], rnd(q[HQ:, 256:384])
                d1 = b1 - t1
                r1 = pltpu.roll(t1, 64, 1)
                st[u]["q"] = (
                    (jnp.where(lo, t0 - b0_, t0).astype(bf16), jnp.where(lo, d1, b0_).astype(bf16),
                     jnp.where(lo, b0_, r1).astype(bf16)),
                    (jnp.where(lo, t2, t2 - b2).astype(bf16), jnp.where(lo, b2, d1).astype(bf16),
                     jnp.where(lo, r1, b2).astype(bf16)))

            def QK(u, j):
                s, i = units[u]
                k = kbuf.at[s, r0 + i]
                ch = lambda n: k[pl.ds(64 * n, 64), :]
                cat = lambda a, b: jnp.concatenate([ch(a), ch(b)], axis=0)
                w1, w2, w3 = (((0, 1), (2, 1), (0, 2)), ((4, 5), (4, 3), (3, 5)))[j]
                l1, l2, l3 = st[u]["q"][j]
                p3 = dot(l3, cat(*w3))
                sc = jnp.concatenate([dot(l1, cat(*w1)) + p3, dot(l2, cat(*w2)) + p3], axis=0)
                m = jnp.max(sc, axis=1, keepdims=True)
                cr = cbuf[s, b0 + i] if norm else c
                p = jnp.exp2((sc - m) * (jnp.concatenate([cr] * 4, axis=1) if norm else cr))
                l = jnp.sum(p, axis=1, keepdims=True)
                r = pl.reciprocal(l, approx=True)
                st[u]["p", j] = (p, r * (2.0 - l * r))

            def PV(u):
                s, i = units[u]
                v = vbuf.at[s, r0 + i]
                (pa, ra), (pb, rb) = st[u]["p", 0], st[u]["p", 1]
                u0 = dot_nt(pa.astype(bf16), v[0:128, :])
                rta = dot_nt(v[128:192, :], pa[:128].astype(bf16))
                u2 = dot_nt(pb.astype(bf16), v[256:384, :])
                rtb = dot_nt(v[192:256, :], pb[:128].astype(bf16))
                cc = dot_nt(jnp.concatenate([pa[128:], pb[128:]], axis=0).astype(bf16), v[128:256, :])
                u1 = jnp.concatenate([jnp.concatenate([rta, rtb], axis=0).T,
                                      jnp.where(lo_mask(32), cc[:32], cc[32:])], axis=0)
                o = jnp.concatenate([u0 * ra, u1 * jnp.where(lo_mask(SQ), ra, rb), u2 * rb], axis=1)
                st[u]["o"] = o.astype(bf16)

            def Op(u):
                s, i = units[u]
                b = b0 + i
                cols = slice(s * D, (s + 1) * D)
                r = dot(st[u]["o"], wobuf[ws, s])
                if first:
                    acc[b, :, cols] = r
                elif last:
                    obuf[b, :, cols] = (acc[b, :, cols] + r).astype(bf16)
                    if s == 1:
                        o_cp(b).start()
                else:
                    acc[b, :, cols] += r

            stage = dict(Q=Qp, A=lambda u: QK(u, 0), B=lambda u: QK(u, 1), V=PV, O=Op)
            for n in range(-5, U + 5):
                for op, off in pat:
                    if 0 <= n + off < U:
                        stage[op](n + off)

        def scoped(name):
            return jax.named_scope(name) if scopes else contextlib.nullcontext()

        def weights(g, op):
            for cp in (wq_cp(g, 0), wq_cp(g, 1), wo_cp(g, 0), wo_cp(g, 1)):
                go(cp, op)

        PRE = R - 1

        def first_items(b, op):
            for s in range(2):
                go(x_cp(b, s), op)
            for w, s in four:
                go(kv_cp(b, 1, w, s), op)

        def issue(j):
            @pl.when(j < B)
            def _():
                first_items(j, "start")

            @pl.when(j == B)
            def _():
                weights(1, "start")

            @pl.when((j >= B + NB - 1) & ((j + 1) % NB == 0))
            def _():
                for w, s in four:
                    kv_cp(j + 1 - NB, NB, w, s).start()

        def first_step(b, _):
            with scoped("f"):
                first_items(b, "wait")
                j = jnp.minimum(2 * b + UP, b + PRE)
                issue(j)
                pl.when(j + 1 <= b + PRE)(lambda: issue(j + 1))
                if norm:
                    for s in range(2):
                        x = xbuf[s, b].astype(f32)
                        a = jnp.max(jnp.abs(x), axis=1, keepdims=True)
                        e = lax.bitcast_convert_type(jnp.clip(a, 2.0 ** -60, 2.0 ** 60), jnp.int32) & 0x7F800000
                        xbuf[s, b] = (x * lax.bitcast_convert_type(0x7F000000 - e, f32)).astype(bf16)
                        cbuf[s, b] = jnp.broadcast_to(lax.bitcast_convert_type(e, f32) * c, (SQ, 128))
                compute(0, b, 1, first=True)

        def big_step(g, cb, last):
            with scoped("l" if last else "m"):
                t = g * B + cb * NB
                for w, s in four:
                    kv_cp(t, NB, w, s).wait()
                nxt = t + R - NB

                def fetch():
                    for w, s in four:
                        kv_cp(nxt, NB, w, s).start()
                if last:
                    pl.when(nxt < NT_)(fetch)
                else:
                    fetch()
                compute(g, cb * NB, NB, last=last)

        def pair(g, last):
            weights(g, "wait")
            if not last:
                weights(g + 1, "start")
            lax.fori_loop(0, B // NB, lambda cb, _: big_step(g, cb, last), None)

        if only:
            lax.fori_loop(0, B // NB, lambda cb, _: compute(1, cb * NB, NB), None)
            return
        weights(0, "start")
        for b in range(UP):
            first_items(b, "start")
        weights(0, "wait")
        lax.fori_loop(0, B, first_step, None)
        lax.fori_loop(1, NP - 1, lambda g, _: pair(g, False), None)
        pair(NP - 1, True)
        for b in range(B):
            o_cp(b).wait()

    hbm = pl.BlockSpec(memory_space=pl.ANY)
    return pl.pallas_call(
        kernel,
        in_specs=[hbm] * 10,
        out_specs=hbm,
        out_shape=jax.ShapeDtypeStruct((B, SQ, 2 * D), jnp.bfloat16),
        scratch_shapes=[
            pltpu.VMEM((2, B, SQ, D), bf16),
            pltpu.VMEM((2, R, PAIR, SK), bf16),
            pltpu.VMEM((2, R, PAIR, SK), bf16),
            pltpu.VMEM((2, 2, D, PAIR), bf16),
            pltpu.VMEM((2, 2, PAIR, D), bf16),
            pltpu.VMEM((B, SQ, 2 * D), f32),
            pltpu.VMEM((B, SQ, 2 * D), bf16),
            pltpu.VMEM((2, B, SQ, 128), f32),
            pltpu.SemaphoreType.DMA((2, B)),
            pltpu.SemaphoreType.DMA((R, 2, 2)),
            pltpu.SemaphoreType.DMA((2, 2)),
            pltpu.SemaphoreType.DMA((2, 2)),
            pltpu.SemaphoreType.DMA((B,)),
        ],
        compiler_params=pltpu.CompilerParams(vmem_limit_bytes=110 * 1024 * 1024, flags=flags,
                                             disable_bounds_checks=nobc),
    )(A_x, tr(A_k), tr(A_v), A_wq, A_wo, B_x, tr(B_k), tr(B_v), B_wq, B_wo)


@jax.jit
def pallas_concat_heads__gqa_block_cached__mha_block_cached__near_ridge_kernel(
        A_x, A_k_cache, A_v_cache, A_wq, A_wo, B_x, B_k_cache, B_v_cache, B_wq, B_wo):
    return build(A_x, A_k_cache, A_v_cache, A_wq, A_wo, B_x, B_k_cache, B_v_cache, B_wq, B_wo)
```

```python
import jax
import jax.numpy as jnp
from jax import lax
import jax.experimental.pallas as pl
import jax.experimental.pallas.tpu as pltpu

B, SQ, D, H, SK, DH = 16, 160, 640, 32, 512, 192
PAIR = 2 * DH
NPAIR = H // 2
HQ = SQ // 2
LOG2E = 1.4426950408889634
f32, bf16 = jnp.float32, jnp.bfloat16

NB_SECOND, NB_MIDDLE, NB_LAST = 4, 8, 2
AHEAD = 5


def _dot(a, b):
    return jnp.dot(a, b, preferred_element_type=f32)


def _dot_nt(a, b):
    return lax.dot_general(a, b, (((1,), (1,)), ((), ())), preferred_element_type=f32)


def _low_lanes(rows):
    return lax.broadcasted_iota(jnp.int32, (rows, 128), 1) < 64


def _project_q(x, wq):
    q = _dot(x, wq)
    lo = _low_lanes(HQ)
    rounded = lambda z: z.astype(bf16).astype(f32)
    t0, t1, t2 = q[:HQ, 0:128], rounded(q[:HQ, 128:256]), q[:HQ, 256:384]
    u0, u1, u2 = rounded(q[HQ:, 0:128]), q[HQ:, 128:256], rounded(q[HQ:, 256:384])
    d1 = u1 - t1
    r1 = pltpu.roll(t1, 64, 1)
    head_a = (jnp.where(lo, t0 - u0, t0), jnp.where(lo, d1, u0), jnp.where(lo, u0, r1))
    head_b = (jnp.where(lo, t2, t2 - u2), jnp.where(lo, u2, d1), jnp.where(lo, r1, u2))
    return tuple(tuple(z.astype(bf16) for z in head) for head in (head_a, head_b))


_KEY_CHUNKS = (((0, 1), (2, 1), (0, 2)), ((4, 5), (4, 3), (3, 5)))


def _softmax_parts(q3, kt_ref, head, scale):
    w_upper, w_lower, w_shared = (
        jnp.concatenate([kt_ref[pl.ds(64 * n, 64), :] for n in chunks], axis=0)
        for chunks in _KEY_CHUNKS[head])
    shared = _dot(q3[2], w_shared)
    s = jnp.concatenate([_dot(q3[0], w_upper) + shared, _dot(q3[1], w_lower) + shared], axis=0)
    m = jnp.max(s, axis=1, keepdims=True)
    p = jnp.exp2((s - m) * jnp.concatenate([scale] * (SK // 128), axis=1))
    l = jnp.sum(p, axis=1, keepdims=True)
    r = pl.reciprocal(l, approx=True)
    return p, r * (2.0 - l * r)


def _weighted_values(pa, ra, pb, rb, vt_ref):
    o0 = _dot_nt(pa.astype(bf16), vt_ref[0:128, :])
    ta = _dot_nt(vt_ref[128:192, :], pa[:128].astype(bf16))
    o2 = _dot_nt(pb.astype(bf16), vt_ref[256:384, :])
    tb = _dot_nt(vt_ref[192:256, :], pb[:128].astype(bf16))
    rest = _dot_nt(jnp.concatenate([pa[128:], pb[128:]], axis=0).astype(bf16), vt_ref[128:256, :])
    n = SQ - 128
    o1 = jnp.concatenate([jnp.concatenate([ta, tb], axis=0).T,
                          jnp.where(_low_lanes(n), rest[:n], rest[n:])], axis=0)
    o = [o0 * ra, o1 * jnp.where(_low_lanes(SQ), ra, rb), o2 * rb]
    return jnp.concatenate(o, axis=1).astype(bf16)


def _start(copies):
    for c in copies:
        c.start()


def _wait(copies):
    for c in copies:
        c.wait()


def _kernel(ax, ak, av, awq, awo, bx, bk, bv, bwq, bwo, out,
            xraw, xbuf, scale, kbuf, vbuf, wqbuf, wobuf, acc, obuf, insem, wsem, osem):
    X, KV, WQ, WO = (ax, bx), ((ak, bk), (av, bv)), (awq, bwq), (awo, bwo)

    def feats(g):
        return pl.ds(g * PAIR if isinstance(g, int) else pl.multiple_of(g * PAIR, 128), PAIR)

    def x_copies(b):
        return [pltpu.make_async_copy(X[s].at[b], xraw.at[s, b], insem.at[(b + B - 1) % B])
                for s in range(2)]

    def kv_copies(g, b0, n, group):
        return [pltpu.make_async_copy(KV[w][s].at[pl.ds(b0, n), feats(g)], buf.at[s, pl.ds(b0, n)],
                                      insem.at[b0 - b0 % group])
                for w, buf in enumerate((kbuf, vbuf)) for s in range(2)]

    def w_copies(g):
        return ([pltpu.make_async_copy(WQ[s].at[:, feats(g)], wqbuf.at[g % 2, s], wsem.at[g % 2])
                 for s in range(2)] +
                [pltpu.make_async_copy(WO[s].at[feats(g)], wobuf.at[g % 2, s], wsem.at[g % 2])
                 for s in range(2)])

    def out_copy(b):
        return pltpu.make_async_copy(obuf.at[b], out.at[b], osem)

    def prepare_x(b):
        for s in range(2):
            x = xraw[s, b].astype(f32)
            top = jnp.clip(jnp.max(jnp.abs(x), axis=1, keepdims=True), 2.0 ** -60, 2.0 ** 60)
            exponent = lax.bitcast_convert_type(top, jnp.int32) & 0x7F800000
            down = lax.bitcast_convert_type(0x7F000000 - exponent, f32)
            up = lax.bitcast_convert_type(exponent, f32)
            xbuf[s, b] = (x * down).astype(bf16)
            scale[s, b] = jnp.broadcast_to(up * (DH ** -0.5 * LOG2E), (SQ, 128))

    def compute(g, b0, nb, mode, caches_read=None):
        units = [(s, b0 + i) for i in range(nb) for s in range(2)]
        q, p, o = {}, {}, {}

        def project(u, s, b):
            q[u] = _project_q(xbuf[s, b], wqbuf[g % 2, s])

        def scores_a(u, s, b):
            p[u] = _softmax_parts(q[u][0], kbuf.at[s, b], 0, scale[s, b])

        def scores_b(u, s, b):
            p[u] += _softmax_parts(q[u][1], kbuf.at[s, b], 1, scale[s, b])

        def values(u, s, b):
            o[u] = _weighted_values(*p[u], vbuf.at[s, b])

        def output(u, s, b):
            cols = slice(s * D, (s + 1) * D)
            r = _dot(o[u], wobuf[g % 2, s])
            if mode == "first":
                acc[b, :, cols] = r
            elif mode == "middle":
                acc[b, :, cols] += r
            else:
                obuf[b, :, cols] = (acc[b, :, cols] + r).astype(bf16)
                if s == 1:
                    out_copy(b).start()

        for n in range(-2, len(units) + 1):
            if caches_read is not None and n == len(units):
                caches_read()
            if mode == "first" and n == 1:
                prepare_x(jnp.minimum(b0 + 1, B - 1))
            for stage, u in ((project, n + 2), (scores_a, n + 1), (values, n),
                             (scores_b, n + 1), (output, n - 1)):
                if 0 <= u < len(units):
                    stage(u, *units[u])

    def first_step(b, _):
        _wait(kv_copies(0, b, 1, 1))
        pl.when(b + 1 < B)(lambda: _wait(x_copies(b + 1)))
        j = b + AHEAD
        pl.when(j + 1 < B)(lambda: _start(x_copies(j + 1)))
        pl.when(j == B)(lambda: _start(w_copies(1)))
        compute(0, b, 1, "first",
                lambda: _start(kv_copies(j // B, j % B, 1, jnp.where(j < B, 1, NB_SECOND))))

    def middle_pair(g, nb):
        _wait(w_copies(g))
        _start(w_copies(g + 1))

        def step(i, _):
            b0 = i * nb
            _wait(kv_copies(g, b0, nb, nb))
            compute(g, b0, nb, "middle", lambda: _start(kv_copies(g + 1, b0, nb, NB_MIDDLE)))

        lax.fori_loop(0, B // nb, step, None)

    def last_step(i, _):
        b0 = i * NB_LAST
        pl.when(b0 % NB_MIDDLE == 0)(
            lambda: _wait(kv_copies(NPAIR - 1, b0, NB_MIDDLE, NB_MIDDLE)))
        compute(NPAIR - 1, b0, NB_LAST, "last")

    _start(x_copies(0) + w_copies(0) + kv_copies(0, 0, 1, 1) + x_copies(1))
    _wait(x_copies(0))
    prepare_x(0)
    _start(kv_copies(0, 1, 1, 1) + x_copies(2))
    _wait(w_copies(0))
    for b in range(2, AHEAD):
        _start(kv_copies(0, b, 1, 1) + x_copies(b + 1))
    lax.fori_loop(0, B, first_step, None)

    aligned = pl.cdiv(AHEAD, NB_SECOND) * NB_SECOND
    for b in range(AHEAD, aligned):
        _start(kv_copies(1, b, 1, NB_SECOND))
    for b in range(aligned, B, NB_SECOND):
        _start(kv_copies(1, b, NB_SECOND, NB_SECOND))
    middle_pair(1, NB_SECOND)
    lax.fori_loop(2, NPAIR - 1, lambda g, _: middle_pair(g, NB_MIDDLE), None)

    _wait(w_copies(NPAIR - 1))
    lax.fori_loop(0, B // NB_LAST, last_step, None)
    _wait([out_copy(b) for b in range(B)])


@jax.jit
def pallas_concat_heads__gqa_block_cached__mha_block_cached__near_ridge_kernel(
    A_x: jax.Array,
    A_k_cache: jax.Array,
    A_v_cache: jax.Array,
    A_wq: jax.Array,
    A_wo: jax.Array,
    B_x: jax.Array,
    B_k_cache: jax.Array,
    B_v_cache: jax.Array,
    B_wq: jax.Array,
    B_wo: jax.Array,
):
    def features_by_keys(cache):
        return jnp.transpose(cache, (0, 1, 3, 2)).reshape(B, H * DH, SK)

    hbm = pl.BlockSpec(memory_space=pl.ANY)
    return pl.pallas_call(
        _kernel,
        in_specs=[hbm] * 10,
        out_specs=hbm,
        out_shape=jax.ShapeDtypeStruct((B, SQ, 2 * D), bf16),
        scratch_shapes=[
            pltpu.VMEM((2, B, SQ, D), bf16),
            pltpu.VMEM((2, B, SQ, D), bf16),
            pltpu.VMEM((2, B, SQ, 128), f32),
            pltpu.VMEM((2, B, PAIR, SK), bf16),
            pltpu.VMEM((2, B, PAIR, SK), bf16),
            pltpu.VMEM((2, 2, D, PAIR), bf16),
            pltpu.VMEM((2, 2, PAIR, D), bf16),
            pltpu.VMEM((B, SQ, 2 * D), f32),
            pltpu.VMEM((B, SQ, 2 * D), bf16),
            pltpu.SemaphoreType.DMA((B,)),
            pltpu.SemaphoreType.DMA((2,)),
            pltpu.SemaphoreType.DMA(()),
        ],
        compiler_params=pltpu.CompilerParams(vmem_limit_bytes=100 * 1024 * 1024),
    )(A_x, features_by_keys(A_k_cache), features_by_keys(A_v_cache), A_wq, A_wo,
      B_x, features_by_keys(B_k_cache), features_by_keys(B_v_cache), B_wq, B_wo)
```

```python
import jax
import jax.numpy as jnp
from jax import lax
import jax.experimental.pallas as pl
import jax.experimental.pallas.tpu as pltpu

B, SQ, D, H, SK, DH = 16, 160, 640, 32, 512, 192
PAIR = 2 * DH
NPAIR = H // 2
HQ = SQ // 2
LOG2E = 1.4426950408889634
f32, bf16 = jnp.float32, jnp.bfloat16

NB_SECOND, NB_MIDDLE, NB_LAST = 4, 8, 2
AHEAD = 5


def _dot(a, b):
    return jnp.dot(a, b, preferred_element_type=f32)


def _dot_nt(a, b):
    return lax.dot_general(a, b, (((1,), (1,)), ((), ())), preferred_element_type=f32)


def _low_lanes(rows):
    return lax.broadcasted_iota(jnp.int32, (rows, 128), 1) < 64


def _project_q(x, wq):
    q = _dot(x, wq)
    lo = _low_lanes(HQ)
    rounded = lambda z: z.astype(bf16).astype(f32)
    t0, t1, t2 = q[:HQ, 0:128], rounded(q[:HQ, 128:256]), q[:HQ, 256:384]
    u0, u1, u2 = rounded(q[HQ:, 0:128]), q[HQ:, 128:256], rounded(q[HQ:, 256:384])
    d1 = u1 - t1
    r1 = pltpu.roll(t1, 64, 1)
    head_a = (jnp.where(lo, t0 - u0, t0), jnp.where(lo, d1, u0), jnp.where(lo, u0, r1))
    head_b = (jnp.where(lo, t2, t2 - u2), jnp.where(lo, u2, d1), jnp.where(lo, r1, u2))
    return tuple(tuple(z.astype(bf16) for z in head) for head in (head_a, head_b))


_KEY_CHUNKS = (((0, 1), (2, 1), (0, 2)), ((4, 5), (4, 3), (3, 5)))


def _softmax_parts(q3, kt_ref, head, scale):
    w_upper, w_lower, w_shared = (
        jnp.concatenate([kt_ref[pl.ds(64 * n, 64), :] for n in chunks], axis=0)
        for chunks in _KEY_CHUNKS[head])
    shared = _dot(q3[2], w_shared)
    s = jnp.concatenate([_dot(q3[0], w_upper) + shared, _dot(q3[1], w_lower) + shared], axis=0)
    m = jnp.max(s, axis=1, keepdims=True)
    p = jnp.exp2((s - m) * jnp.concatenate([scale] * (SK // 128), axis=1))
    return p, jnp.sum(p, axis=1, keepdims=True)


def _weighted_values(pa, la, pb, lb, vt_ref):
    o0 = _dot_nt(pa.astype(bf16), vt_ref[0:128, :])
    ta = _dot_nt(vt_ref[128:192, :], pa[:128].astype(bf16))
    o2 = _dot_nt(pb.astype(bf16), vt_ref[256:384, :])
    tb = _dot_nt(vt_ref[192:256, :], pb[:128].astype(bf16))
    rest = _dot_nt(jnp.concatenate([pa[128:], pb[128:]], axis=0).astype(bf16), vt_ref[128:256, :])
    n = SQ - 128
    o1 = jnp.concatenate([jnp.concatenate([ta, tb], axis=0).T,
                          jnp.where(_low_lanes(n), rest[:n], rest[n:])], axis=0)
    lo = _low_lanes(SQ)
    r = 1.0 / jnp.where(lo, la, lb)
    swapped = pltpu.roll(r, 64, 1)
    o = [o0 * jnp.where(lo, r, swapped), o1 * r, o2 * jnp.where(lo, swapped, r)]
    return jnp.concatenate(o, axis=1).astype(bf16)


def _start(copies):
    for c in copies:
        c.start()


def _wait(copies):
    for c in copies:
        c.wait()


def _kernel(ax, ak, av, awq, awo, bx, bk, bv, bwq, bwo, out,
            xraw, xbuf, scale, kbuf, vbuf, wqbuf, wobuf, acc, obuf, insem, wsem, osem):
    X, KV, WQ, WO = (ax, bx), ((ak, bk), (av, bv)), (awq, bwq), (awo, bwo)

    def feats(g):
        return pl.ds(g * PAIR if isinstance(g, int) else pl.multiple_of(g * PAIR, 128), PAIR)

    def x_copies(b):
        return [pltpu.make_async_copy(X[s].at[b], xraw.at[s, b], insem.at[(b + B - 1) % B])
                for s in range(2)]

    def kv_copies(g, b0, n, group):
        return [pltpu.make_async_copy(KV[w][s].at[pl.ds(b0, n), feats(g)], buf.at[s, pl.ds(b0, n)],
                                      insem.at[b0 - b0 % group])
                for w, buf in enumerate((kbuf, vbuf)) for s in range(2)]

    def w_copies(g):
        return ([pltpu.make_async_copy(WQ[s].at[:, feats(g)], wqbuf.at[g % 2, s], wsem.at[g % 2])
                 for s in range(2)] +
                [pltpu.make_async_copy(WO[s].at[feats(g)], wobuf.at[g % 2, s], wsem.at[g % 2])
                 for s in range(2)])

    def out_copy(b):
        return pltpu.make_async_copy(obuf.at[b], out.at[b], osem)

    def prepare_x(b):
        for s in range(2):
            x = xraw[s, b].astype(f32)
            top = jnp.clip(jnp.max(jnp.abs(x), axis=1, keepdims=True), 2.0 ** -60, 2.0 ** 60)
            exponent = lax.bitcast_convert_type(top, jnp.int32) & 0x7F800000
            down = lax.bitcast_convert_type(0x7F000000 - exponent, f32)
            up = lax.bitcast_convert_type(exponent, f32)
            xbuf[s, b] = (x * down).astype(bf16)
            scale[s, b] = jnp.broadcast_to(up * (DH ** -0.5 * LOG2E), (SQ, 128))

    def compute(g, b0, nb, mode, caches_read=None):
        units = [(s, b0 + i) for i in range(nb) for s in range(2)]
        q, p, o = {}, {}, {}

        def project(u, s, b):
            q[u] = _project_q(xbuf[s, b], wqbuf[g % 2, s])

        def scores_a(u, s, b):
            p[u] = _softmax_parts(q[u][0], kbuf.at[s, b], 0, scale[s, b])

        def scores_b(u, s, b):
            p[u] += _softmax_parts(q[u][1], kbuf.at[s, b], 1, scale[s, b])

        def values(u, s, b):
            o[u] = _weighted_values(*p[u], vbuf.at[s, b])

        def output(u, s, b):
            cols = slice(s * D, (s + 1) * D)
            r = _dot(o[u], wobuf[g % 2, s])
            if mode == "first":
                acc[b, :, cols] = r
            elif mode == "middle":
                acc[b, :, cols] += r
            else:
                obuf[b, :, cols] = (acc[b, :, cols] + r).astype(bf16)
                if s == 1:
                    out_copy(b).start()

        pipeline = [(project, 2), (scores_a, 1), (values, 0), (scores_b, 1), (output, -1)]
        if nb == 1:
            pipeline[2], pipeline[3] = pipeline[3], pipeline[2]
        for n in range(-2, len(units) + 1):
            if caches_read is not None and n == len(units):
                caches_read()
            if mode == "first" and n == 1:
                prepare_x(jnp.minimum(b0 + 1, B - 1))
            for stage, ahead in pipeline:
                if 0 <= n + ahead < len(units):
                    stage(n + ahead, *units[n + ahead])

    def first_step(b, _):
        _wait(kv_copies(0, b, 1, 1))
        pl.when(b + 1 < B)(lambda: _wait(x_copies(b + 1)))
        j = b + AHEAD
        pl.when(j + 1 < B)(lambda: _start(x_copies(j + 1)))
        pl.when(j == B)(lambda: _start(w_copies(1)))
        compute(0, b, 1, "first",
                lambda: _start(kv_copies(j // B, j % B, 1, jnp.where(j < B, 1, NB_SECOND))))

    def middle_pair(g, nb):
        _wait(w_copies(g))
        _start(w_copies(g + 1))

        def step(i, _):
            b0 = i * nb
            _wait(kv_copies(g, b0, nb, nb))
            compute(g, b0, nb, "middle", lambda: _start(kv_copies(g + 1, b0, nb, NB_MIDDLE)))

        lax.fori_loop(0, B // nb, step, None)

    def last_step(i, _):
        b0 = i * NB_LAST
        pl.when(b0 % NB_MIDDLE == 0)(
            lambda: _wait(kv_copies(NPAIR - 1, b0, NB_MIDDLE, NB_MIDDLE)))
        compute(NPAIR - 1, b0, NB_LAST, "last")

    _start(x_copies(0) + w_copies(0) + kv_copies(0, 0, 1, 1) + x_copies(1))
    _wait(x_copies(0))
    prepare_x(0)
    _start(kv_copies(0, 1, 1, 1) + x_copies(2))
    _wait(w_copies(0))
    for b in range(2, AHEAD):
        _start(kv_copies(0, b, 1, 1) + x_copies(b + 1))
    lax.fori_loop(0, B, first_step, None)

    aligned = pl.cdiv(AHEAD, NB_SECOND) * NB_SECOND
    for b in range(AHEAD, aligned):
        _start(kv_copies(1, b, 1, NB_SECOND))
    for b in range(aligned, B, NB_SECOND):
        _start(kv_copies(1, b, NB_SECOND, NB_SECOND))
    middle_pair(1, NB_SECOND)
    lax.fori_loop(2, NPAIR - 1, lambda g, _: middle_pair(g, NB_MIDDLE), None)

    _wait(w_copies(NPAIR - 1))
    lax.fori_loop(0, B // NB_LAST, last_step, None)
    _wait([out_copy(b) for b in range(B)])


@jax.jit
def pallas_concat_heads__gqa_block_cached__mha_block_cached__near_ridge_kernel(
    A_x: jax.Array,
    A_k_cache: jax.Array,
    A_v_cache: jax.Array,
    A_wq: jax.Array,
    A_wo: jax.Array,
    B_x: jax.Array,
    B_k_cache: jax.Array,
    B_v_cache: jax.Array,
    B_wq: jax.Array,
    B_wo: jax.Array,
):
    def features_by_keys(cache):
        return jnp.transpose(cache, (0, 1, 3, 2)).reshape(B, H * DH, SK)

    hbm = pl.BlockSpec(memory_space=pl.ANY)
    return pl.pallas_call(
        _kernel,
        in_specs=[hbm] * 10,
        out_specs=hbm,
        out_shape=jax.ShapeDtypeStruct((B, SQ, 2 * D), bf16),
        scratch_shapes=[
            pltpu.VMEM((2, B, SQ, D), bf16),
            pltpu.VMEM((2, B, SQ, D), bf16),
            pltpu.VMEM((2, B, SQ, 128), f32),
            pltpu.VMEM((2, B, PAIR, SK), bf16),
            pltpu.VMEM((2, B, PAIR, SK), bf16),
            pltpu.VMEM((2, 2, D, PAIR), bf16),
            pltpu.VMEM((2, 2, PAIR, D), bf16),
            pltpu.VMEM((B, SQ, 2 * D), f32),
            pltpu.VMEM((B, SQ, 2 * D), bf16),
            pltpu.SemaphoreType.DMA((B,)),
            pltpu.SemaphoreType.DMA((2,)),
            pltpu.SemaphoreType.DMA(()),
        ],
        compiler_params=pltpu.CompilerParams(vmem_limit_bytes=100 * 1024 * 1024),
    )(A_x, features_by_keys(A_k_cache), features_by_keys(A_v_cache), A_wq, A_wo,
      B_x, features_by_keys(B_k_cache), features_by_keys(B_v_cache), B_wq, B_wo)
```

```python
import jax
import jax.numpy as jnp
from jax import lax
import jax.experimental.pallas as pl
import jax.experimental.pallas.tpu as pltpu

B, SQ, D, H, SK, DH = 16, 160, 640, 32, 512, 192
PAIR = 2 * DH
NPAIR = H // 2
HQ = SQ // 2
SCALE = DH ** -0.5 * 1.4426950408889634
f32, bf16, i32 = jnp.float32, jnp.bfloat16, jnp.int32

MAX_SPLIT_ERROR = 2.0 ** -4

NB_SECOND, NB_MIDDLE, NB_LAST = 4, 8, 2
AHEAD = 5


def _dot(a, b):
    return jnp.dot(a, b, preferred_element_type=f32)


def _dot_nt(a, b):
    return lax.dot_general(a, b, (((1,), (1,)), ((), ())), preferred_element_type=f32)


def _low_lanes(rows):
    return lax.broadcasted_iota(i32, (rows, 128), 1) < 64


def _fold_tiles(op, z):
    parts = [z[i:i + 8, j:j + 128]
             for i in range(0, z.shape[0], 8) for j in range(0, z.shape[1], 128)]
    while len(parts) > 1:
        parts = [op(parts[i], parts[i + 1]) if i + 1 < len(parts) else parts[i]
                 for i in range(0, len(parts), 2)]
    return parts[0]


def _split_queries(q):
    full, lo = _low_lanes(SQ), _low_lanes(HQ)
    e = lax.bitcast_convert_type(lax.bitcast_convert_type(q, i32) & 0x7F800000, f32)
    top = lambda z: jnp.clip(jnp.max(z, axis=1, keepdims=True), 2.0 ** -126, 2.0 ** 126)
    inverse = lambda z: lax.bitcast_convert_type(
        0x7F000000 - lax.bitcast_convert_type(z, i32), f32)
    up_a = top(jnp.maximum(e[:, 0:128], jnp.where(full, e[:, 128:256], 0.0)))
    up_b = top(jnp.maximum(e[:, 256:384], jnp.where(full, 0.0, e[:, 128:256])))
    down_a, down_b = inverse(up_a), inverse(up_b)
    down = jnp.where(full, down_a, down_b)
    q0, q1, q2 = q[:, 0:128] * down_a, q[:, 128:256] * down, q[:, 256:384] * down_b

    rounded = lambda z: z.astype(bf16).astype(f32)
    t0, t1, t2 = q0[:HQ], rounded(q1[:HQ]), q2[:HQ]
    u0, u1, u2 = rounded(q0[HQ:]), q1[HQ:], rounded(q2[HQ:])
    d0 = jnp.where(lo, t0 - u0, t2 - u2)
    d1 = u1 - t1
    r1 = pltpu.roll(t1, 64, 1)
    head_a = (jnp.where(lo, d0, t0), jnp.where(lo, d1, u0), jnp.where(lo, u0, r1))
    head_b = (jnp.where(lo, t2, d0), jnp.where(lo, u2, d1), jnp.where(lo, r1, u2))

    d = jnp.concatenate([d0, d1], axis=0)
    lost = jnp.abs(rounded(d) - d)
    lost = jnp.where(full, jnp.sum(jnp.where(full, lost, 0.0), axis=1, keepdims=True),
                     jnp.sum(jnp.where(full, 0.0, lost), axis=1, keepdims=True))
    return ((tuple(z.astype(bf16) for z in head_a), up_a * SCALE),
            (tuple(z.astype(bf16) for z in head_b), up_b * SCALE), lost, down)


_KEY_CHUNKS = (((0, 1), (2, 1), (0, 2)), ((4, 5), (4, 3), (3, 5)))


def _split_scores(q3, kt_ref, head):
    k_upper, k_lower, k_shared = (
        jnp.concatenate([kt_ref[pl.ds(64 * n, 64), :] for n in chunks], axis=0)
        for chunks in _KEY_CHUNKS[head])
    shared = _dot(q3[2], k_shared)
    s = jnp.concatenate([_dot(q3[0], k_upper) + shared, _dot(q3[1], k_lower) + shared], axis=0)
    pairs = pltpu.bitcast(k_shared, i32) & 0x7FFF7FFF
    largest = _fold_tiles(jnp.maximum, jnp.maximum(lax.bitcast_convert_type(pairs, f32),
                                                   lax.bitcast_convert_type(pairs << 16, f32)))
    return s, jnp.max(jnp.max(largest, axis=1, keepdims=True), axis=0, keepdims=True)


def _plain_scores(q, kt_ref, head):
    lo, middle = _low_lanes(SQ), q[:, 128:256]
    k, zero = kt_ref[pl.ds(DH * head, DH), :], jnp.zeros((64, SK), bf16)
    if head == 0:
        qs, ks = [q[:, 0:128], jnp.where(lo, middle, 0.0)], [k, zero]
    else:
        qs, ks = [jnp.where(lo, 0.0, middle), q[:, 256:384]], [zero, k]
    return _dot(jnp.concatenate(qs, axis=1).astype(bf16), jnp.concatenate(ks, axis=0))


def _softmax_parts(s, scale):
    m = jnp.max(s, axis=1, keepdims=True)
    p = jnp.exp2((s - m) * scale)
    return p, jnp.sum(p, axis=1, keepdims=True), m


def _weighted_values(pa, pb, l, vt_ref):
    o0 = _dot_nt(pa.astype(bf16), vt_ref[0:128, :])
    ta = _dot_nt(vt_ref[128:192, :], pa[:128].astype(bf16))
    o2 = _dot_nt(pb.astype(bf16), vt_ref[256:384, :])
    tb = _dot_nt(vt_ref[192:256, :], pb[:128].astype(bf16))
    rest = _dot_nt(jnp.concatenate([pa[128:], pb[128:]], axis=0).astype(bf16), vt_ref[128:256, :])
    n = SQ - 128
    o1 = jnp.concatenate([jnp.concatenate([ta, tb], axis=0).T,
                          jnp.where(_low_lanes(n), rest[:n], rest[n:])], axis=0)
    lo = _low_lanes(SQ)
    r = 1.0 / l
    swapped = pltpu.roll(r, 64, 1)
    o = [o0 * jnp.where(lo, r, swapped), o1 * r, o2 * jnp.where(lo, swapped, r)]
    return jnp.concatenate(o, axis=1).astype(bf16)


def _start(copies):
    for c in copies:
        c.start()


def _wait(copies):
    for c in copies:
        c.wait()


def _kernel(ax, ak, av, awq, awo, bx, bk, bv, bwq, bwo, out,
            xbuf, kbuf, vbuf, wqbuf, wobuf, acc, obuf, probe, insem, wsem, osem):
    X, KV, WQ, WO = (ax, bx), ((ak, bk), (av, bv)), (awq, bwq), (awo, bwo)

    def feats(g):
        return pl.ds(g * PAIR if isinstance(g, int) else pl.multiple_of(g * PAIR, 128), PAIR)

    def x_copies(b):
        return [pltpu.make_async_copy(X[s].at[b], xbuf.at[s, b], insem.at[b]) for s in range(2)]

    def kv_copies(g, b0, n, group):
        return [pltpu.make_async_copy(KV[w][s].at[pl.ds(b0, n), feats(g)], buf.at[s, pl.ds(b0, n)],
                                      insem.at[b0 - b0 % group])
                for w, buf in enumerate((kbuf, vbuf)) for s in range(2)]

    def w_copies(g):
        return ([pltpu.make_async_copy(WQ[s].at[:, feats(g)], wqbuf.at[g % 2, s], wsem.at[g % 2])
                 for s in range(2)] +
                [pltpu.make_async_copy(WO[s].at[feats(g)], wobuf.at[g % 2, s], wsem.at[g % 2])
                 for s in range(2)])

    def out_copy(b):
        return pltpu.make_async_copy(obuf.at[b], out.at[b], osem)

    def compute(g, b0, nb, mode, caches_read=None, plain=False):
        units = [(s, b0 + i) for i in range(nb) for s in range(2)]
        q, p, largest, o = {}, {}, {}, {}

        def project(u, s, b):
            q[u] = _dot(xbuf[s, b], wqbuf[g % 2, s])
            if not plain:
                q[u] = _split_queries(q[u])

        def scores(head, u, s, b):
            if plain:
                p[u, head] = _softmax_parts(_plain_scores(q[u], kbuf.at[s, b], head), SCALE)
            else:
                q3, scale = q[u][head]
                z, largest[u, head] = _split_scores(q3, kbuf.at[s, b], head)
                p[u, head] = _softmax_parts(z, scale)

        def values(u, s, b):
            (pa, la, ma), (pb, lb, mb) = p[u, 0], p[u, 1]
            lo = _low_lanes(SQ)
            l = jnp.where(lo, la, lb)
            if not plain:
                lost, down = q[u][2:]
                k = jnp.where(_low_lanes(1), largest[u, 0], largest[u, 1])
                top = jnp.maximum(jnp.abs(jnp.where(lo, ma, mb)), down)
                l = jnp.where(lost * (k * (1.0 / MAX_SPLIT_ERROR)) <= top, l, jnp.nan)
            o[u] = _weighted_values(pa, pb, l, vbuf.at[s, b])

        def output(u, s, b):
            cols = slice(s * D, (s + 1) * D)
            r = _dot(o[u], wobuf[g % 2, s])
            if mode == "first":
                acc[b, :, cols] = r
            elif mode == "middle":
                acc[b, :, cols] += r
            else:
                r = acc[b, :, cols] + r
                obuf[b, :, cols] = r.astype(bf16)
                probe[...] += _fold_tiles(jnp.add, r[:, 0:128])
                if s == 1:
                    out_copy(b).start()

        scores_a = lambda *args: scores(0, *args)
        scores_b = lambda *args: scores(1, *args)
        for n in range(-2, len(units) + 1):
            if caches_read is not None and n == len(units):
                caches_read()
            stages = [(project, 2), (scores_a, 1), (values, 0), (scores_b, 1), (output, -1)]
            if nb <= 2 and n + 2 >= len(units):
                stages[2], stages[3] = stages[3], stages[2]
            for stage, ahead in stages:
                if 0 <= n + ahead < len(units):
                    stage(n + ahead, *units[n + ahead])

    def first_step(b, _):
        _wait(x_copies(b) + kv_copies(0, b, 1, 1))
        j = b + AHEAD
        pl.when(j < B)(lambda: _start(x_copies(j)))
        pl.when(j == B)(lambda: _start(w_copies(1)))
        compute(0, b, 1, "first",
                lambda: _start(kv_copies(j // B, j % B, 1, jnp.where(j < B, 1, NB_SECOND))))

    def middle_pair(g, nb):
        _wait(w_copies(g))
        _start(w_copies(g + 1))

        def step(i, _):
            b0 = i * nb
            _wait(kv_copies(g, b0, nb, nb))
            compute(g, b0, nb, "middle", lambda: _start(kv_copies(g + 1, b0, nb, NB_MIDDLE)))

        lax.fori_loop(0, B // nb, step, None)

    def last_step(i, _):
        b0 = i * NB_LAST
        pl.when(b0 % NB_MIDDLE == 0)(
            lambda: _wait(kv_copies(NPAIR - 1, b0, NB_MIDDLE, NB_MIDDLE)))
        compute(NPAIR - 1, b0, NB_LAST, "last")

    _start(w_copies(0))
    for b in range(2):
        _start(x_copies(b) + kv_copies(0, b, 1, 1))
    probe[...] = jnp.zeros_like(probe)
    _wait(w_copies(0))
    for b in range(2, AHEAD):
        _start(x_copies(b) + kv_copies(0, b, 1, 1))
    lax.fori_loop(0, B, first_step, None)

    aligned = pl.cdiv(AHEAD, NB_SECOND) * NB_SECOND
    for b in range(AHEAD, aligned):
        _start(kv_copies(1, b, 1, NB_SECOND))
    for b in range(aligned, B, NB_SECOND):
        _start(kv_copies(1, b, NB_SECOND, NB_SECOND))
    middle_pair(1, NB_SECOND)
    lax.fori_loop(2, NPAIR - 1, lambda g, _: middle_pair(g, NB_MIDDLE), None)

    _wait(w_copies(NPAIR - 1))
    lax.fori_loop(0, B // NB_LAST, last_step, None)
    saw_nan = jnp.sum(jnp.where(probe[...] == probe[...], 0.0, 1.0)) > 0.0
    _wait([out_copy(b) for b in range(B)])

    @pl.when(saw_nan)
    def _recompute_with_plain_scores():
        def clear(b, _):
            _start(kv_copies(0, b, 1, 1))
            acc[b] = jnp.zeros((SQ, 2 * D), f32)

        def pair(g, _):
            _wait(w_copies(g))
            pl.when(g + 1 < NPAIR)(lambda: _start(w_copies(g + 1)))

            def step(b, _):
                _wait(kv_copies(g, b, 1, 1))
                compute(g, b, 1, "middle", plain=True)
                pl.when(g + 1 < NPAIR)(lambda: _start(kv_copies(g + 1, b, 1, 1)))

            lax.fori_loop(0, B, step, None)

        def store(b, _):
            obuf[b] = acc[b].astype(bf16)
            out_copy(b).start()

        _start(w_copies(0))
        lax.fori_loop(0, B, clear, None)
        lax.fori_loop(0, NPAIR, pair, None)
        lax.fori_loop(0, B, store, None)
        _wait([out_copy(b) for b in range(B)])


@jax.jit
def pallas_concat_heads__gqa_block_cached__mha_block_cached__near_ridge_kernel(
    A_x: jax.Array,
    A_k_cache: jax.Array,
    A_v_cache: jax.Array,
    A_wq: jax.Array,
    A_wo: jax.Array,
    B_x: jax.Array,
    B_k_cache: jax.Array,
    B_v_cache: jax.Array,
    B_wq: jax.Array,
    B_wo: jax.Array,
):
    def features_by_keys(cache):
        return jnp.transpose(cache, (0, 1, 3, 2)).reshape(B, H * DH, SK)

    hbm = pl.BlockSpec(memory_space=pl.ANY)
    return pl.pallas_call(
        _kernel,
        in_specs=[hbm] * 10,
        out_specs=hbm,
        out_shape=jax.ShapeDtypeStruct((B, SQ, 2 * D), bf16),
        scratch_shapes=[
            pltpu.VMEM((2, B, SQ, D), bf16),
            pltpu.VMEM((2, B, PAIR, SK), bf16),
            pltpu.VMEM((2, B, PAIR, SK), bf16),
            pltpu.VMEM((2, 2, D, PAIR), bf16),
            pltpu.VMEM((2, 2, PAIR, D), bf16),
            pltpu.VMEM((B, SQ, 2 * D), f32),
            pltpu.VMEM((B, SQ, 2 * D), bf16),
            pltpu.VMEM((8, 128), f32),
            pltpu.SemaphoreType.DMA((B,)),
            pltpu.SemaphoreType.DMA((2,)),
            pltpu.SemaphoreType.DMA(()),
        ],
        compiler_params=pltpu.CompilerParams(vmem_limit_bytes=100 * 1024 * 1024),
    )(A_x, features_by_keys(A_k_cache), features_by_keys(A_v_cache), A_wq, A_wo,
      B_x, features_by_keys(B_k_cache), features_by_keys(B_v_cache), B_wq, B_wo)
```

```python
import jax
import jax.numpy as jnp
from jax import lax
import jax.experimental.pallas as pl
import jax.experimental.pallas.tpu as pltpu

B, SQ, D, H, SK, DH = 16, 160, 640, 32, 512, 192
PAIR = 2 * DH
NPAIR = H // 2
HQ = SQ // 2
SCALE = DH ** -0.5 * 1.4426950408889634
f32, bf16, i32 = jnp.float32, jnp.bfloat16, jnp.int32

MAX_SPLIT_ERROR = 2.0 ** -4

NB_SECOND, NB_MIDDLE, NB_LAST = 2, 8, 2
AHEAD = 4


def _dot(a, b):
    return jnp.dot(a, b, preferred_element_type=f32)


def _dot_nt(a, b):
    return lax.dot_general(a, b, (((1,), (1,)), ((), ())), preferred_element_type=f32)


def _low_lanes(rows):
    return lax.broadcasted_iota(i32, (rows, 128), 1) < 64


def _fold_tiles(op, z):
    parts = [z[i:i + 8, j:j + 128]
             for i in range(0, z.shape[0], 8) for j in range(0, z.shape[1], 128)]
    while len(parts) > 1:
        parts = [op(parts[i], parts[i + 1]) if i + 1 < len(parts) else parts[i]
                 for i in range(0, len(parts), 2)]
    return parts[0]


def _split_queries(q):
    full, lo = _low_lanes(SQ), _low_lanes(HQ)
    e = lax.bitcast_convert_type(lax.bitcast_convert_type(q, i32) & 0x7F800000, f32)
    top = lambda z: jnp.clip(jnp.max(z, axis=1, keepdims=True), 2.0 ** -126, 2.0 ** 126)
    inverse = lambda z: lax.bitcast_convert_type(
        0x7F000000 - lax.bitcast_convert_type(z, i32), f32)
    up_a = top(jnp.maximum(e[:, 0:128], jnp.where(full, e[:, 128:256], 0.0)))
    up_b = top(jnp.maximum(e[:, 256:384], jnp.where(full, 0.0, e[:, 128:256])))
    down_a, down_b = inverse(up_a), inverse(up_b)
    down = jnp.where(full, down_a, down_b)
    q0, q1, q2 = q[:, 0:128] * down_a, q[:, 128:256] * down, q[:, 256:384] * down_b

    rounded = lambda z: z.astype(bf16).astype(f32)
    t0, t1, t2 = q0[:HQ], rounded(q1[:HQ]), q2[:HQ]
    u0, u1, u2 = rounded(q0[HQ:]), q1[HQ:], rounded(q2[HQ:])
    d0 = jnp.where(lo, t0 - u0, t2 - u2)
    d1 = u1 - t1
    r1 = pltpu.roll(t1, 64, 1)
    head_a = (jnp.where(lo, d0, t0), jnp.where(lo, d1, u0), jnp.where(lo, u0, r1))
    head_b = (jnp.where(lo, t2, d0), jnp.where(lo, u2, d1), jnp.where(lo, r1, u2))

    d = jnp.concatenate([d0, d1], axis=0)
    lost = jnp.abs(rounded(d) - d)
    f32_slack = 2.0 ** -22
    lost = jnp.where(full, jnp.sum(jnp.where(full, lost, f32_slack), axis=1, keepdims=True),
                     jnp.sum(jnp.where(full, f32_slack, lost), axis=1, keepdims=True))
    return ((tuple(z.astype(bf16) for z in head_a), up_a * SCALE),
            (tuple(z.astype(bf16) for z in head_b), up_b * SCALE), lost, down)


_KEY_CHUNKS = (((0, 1), (2, 1), (0, 2)), ((4, 5), (4, 3), (3, 5)))


def _split_scores(q3, kt_ref, head):
    k_upper, k_lower, k_shared = (
        jnp.concatenate([kt_ref[pl.ds(64 * n, 64), :] for n in chunks], axis=0)
        for chunks in _KEY_CHUNKS[head])
    shared = _dot(q3[2], k_shared)
    s = jnp.concatenate([_dot(q3[0], k_upper) + shared, _dot(q3[1], k_lower) + shared], axis=0)
    pairs = pltpu.bitcast(k_shared, i32) & 0x7FFF7FFF
    largest = _fold_tiles(jnp.maximum, jnp.maximum(lax.bitcast_convert_type(pairs, f32),
                                                   lax.bitcast_convert_type(pairs << 16, f32)))
    return s, jnp.max(jnp.max(largest, axis=1, keepdims=True), axis=0, keepdims=True)


def _plain_scores(q, kt_ref, head):
    lo, middle = _low_lanes(SQ), q[:, 128:256]
    k, zero = kt_ref[pl.ds(DH * head, DH), :], jnp.zeros((64, SK), bf16)
    if head == 0:
        qs, ks = [q[:, 0:128], jnp.where(lo, middle, 0.0)], [k, zero]
    else:
        qs, ks = [jnp.where(lo, 0.0, middle), q[:, 256:384]], [zero, k]
    return _dot(jnp.concatenate(qs, axis=1).astype(bf16), jnp.concatenate(ks, axis=0))


def _softmax_parts(s, scale):
    m = jnp.max(s, axis=1, keepdims=True)
    p = jnp.exp2((s - m) * scale)
    return p, jnp.sum(p, axis=1, keepdims=True), m


def _weighted_values(pa, pb, l, vt_ref):
    o0 = _dot_nt(pa.astype(bf16), vt_ref[0:128, :])
    ta = _dot_nt(vt_ref[128:192, :], pa[:128].astype(bf16))
    o2 = _dot_nt(pb.astype(bf16), vt_ref[256:384, :])
    tb = _dot_nt(vt_ref[192:256, :], pb[:128].astype(bf16))
    rest = _dot_nt(jnp.concatenate([pa[128:], pb[128:]], axis=0).astype(bf16), vt_ref[128:256, :])
    n = SQ - 128
    o1 = jnp.concatenate([jnp.concatenate([ta, tb], axis=0).T,
                          jnp.where(_low_lanes(n), rest[:n], rest[n:])], axis=0)
    lo = _low_lanes(SQ)
    r = 1.0 / l
    swapped = pltpu.roll(r, 64, 1)
    o = [o0 * jnp.where(lo, r, swapped), o1 * r, o2 * jnp.where(lo, swapped, r)]
    return jnp.concatenate(o, axis=1).astype(bf16)


def _stage_order(n_units, mode):
    if n_units == 2:
        order = "Q0 Q1 B0 A0 A1 B1 V0 V1 O0 O1".split()
    elif n_units == 4 and mode == "last":
        order = "Q0 Q1 B0 A0 Q2 A1 V0 B1 A2 Q3 B2 V1 B3 O0 A3 V2 O1 V3 O2 O3".split()
    elif n_units == 4:
        order = "Q0 Q1 A0 B0 Q2 A1 B1 V0 B2 A2 Q3 O0 V1 A3 B3 O1 V2 V3 O2 O3".split()
    else:
        order = [f"{stage}{n + ahead}" for n in range(-2, n_units + 1)
                 for stage, ahead in (("Q", 2), ("A", 1), ("V", 0), ("B", 1), ("O", -1))
                 if 0 <= n + ahead < n_units]
        for early in ("V0", f"Q{n_units - 1}", f"B{n_units - 2}"):
            i = order.index(early)
            order[i - 1], order[i] = order[i], order[i - 1]
    return [(z[0], int(z[1:])) for z in order]


def _start(copies):
    for c in copies:
        c.start()


def _wait(copies):
    for c in copies:
        c.wait()


def _kernel(ax, ak, av, awq, awo, bx, bk, bv, bwq, bwo, out,
            xbuf, kbuf, vbuf, wqbuf, wobuf, acc, obuf, probe, insem, wsem, osem):
    X, KV, WQ, WO = (ax, bx), ((ak, bk), (av, bv)), (awq, bwq), (awo, bwo)

    def feats(g):
        return pl.ds(g * PAIR if isinstance(g, int) else pl.multiple_of(g * PAIR, 128), PAIR)

    def x_copies(b):
        return [pltpu.make_async_copy(X[s].at[b], xbuf.at[s, b], insem.at[b]) for s in range(2)]

    def kv_copies(g, b0, n, group):
        return [pltpu.make_async_copy(KV[w][s].at[pl.ds(b0, n), feats(g)], buf.at[s, pl.ds(b0, n)],
                                      insem.at[b0 - b0 % group])
                for w, buf in enumerate((kbuf, vbuf)) for s in range(2)]

    def w_copies(g):
        return ([pltpu.make_async_copy(WQ[s].at[:, feats(g)], wqbuf.at[g % 2, s], wsem.at[g % 2])
                 for s in range(2)] +
                [pltpu.make_async_copy(WO[s].at[feats(g)], wobuf.at[g % 2, s], wsem.at[g % 2])
                 for s in range(2)])

    def out_copy(b):
        return pltpu.make_async_copy(obuf.at[b], out.at[b], osem)

    def compute(g, b0, nb, mode, caches_read=None, plain=False):
        units = [(s, b0 + i) for i in range(nb) for s in range(2)]
        q, p, largest, o = {}, {}, {}, {}

        def project(u, s, b):
            q[u] = _dot(xbuf[s, b], wqbuf[g % 2, s])
            if not plain:
                q[u] = _split_queries(q[u])

        def scores(head, u, s, b):
            if plain:
                p[u, head] = _softmax_parts(_plain_scores(q[u], kbuf.at[s, b], head), SCALE)
            else:
                q3, scale = q[u][head]
                z, largest[u, head] = _split_scores(q3, kbuf.at[s, b], head)
                p[u, head] = _softmax_parts(z, scale)

        def values(u, s, b):
            (pa, la, ma), (pb, lb, mb) = p[u, 0], p[u, 1]
            lo = _low_lanes(SQ)
            l = jnp.where(lo, la, lb)
            if not plain:
                lost, down = q[u][2:]
                k = jnp.where(_low_lanes(1), largest[u, 0], largest[u, 1])
                top = jnp.maximum(jnp.abs(jnp.where(lo, ma, mb)), down)
                l = jnp.where(lost * (k * (1.0 / MAX_SPLIT_ERROR)) <= top, l, jnp.nan)
            o[u] = _weighted_values(pa, pb, l, vbuf.at[s, b])

        def output(u, s, b):
            cols = slice(s * D, (s + 1) * D)
            r = _dot(o[u], wobuf[g % 2, s])
            if mode == "first":
                acc[b, :, cols] = r
            elif mode == "middle":
                acc[b, :, cols] += r
            else:
                r = acc[b, :, cols] + r
                obuf[b, :, cols] = r.astype(bf16)
                probe[...] += _fold_tiles(jnp.add, r[:, 0:128])
                if s == 1:
                    out_copy(b).start()

        stages = dict(Q=project, A=lambda *args: scores(0, *args),
                      B=lambda *args: scores(1, *args), V=values, O=output)
        order = _stage_order(len(units), mode)
        for n, (stage, u) in enumerate(order):
            if caches_read is not None and n == len(order) - 1:
                caches_read()
            stages[stage](u, *units[u])

    def first_step(b, _):
        _wait(x_copies(b) + kv_copies(0, b, 1, 1))
        j = b + AHEAD
        pl.when(j < B)(lambda: _start(x_copies(j)))
        pl.when(j == B)(lambda: _start(w_copies(1)))
        compute(0, b, 1, "first",
                lambda: _start(kv_copies(j // B, j % B, 1, jnp.where(j < B, 1, NB_SECOND))))

    def middle_pair(g, nb):
        _wait(w_copies(g))
        _start(w_copies(g + 1))

        def step(i, _):
            b0 = i * nb
            _wait(kv_copies(g, b0, nb, nb))
            compute(g, b0, nb, "middle", lambda: _start(kv_copies(g + 1, b0, nb, NB_MIDDLE)))

        lax.fori_loop(0, B // nb, step, None)

    def last_step(i, _):
        b0 = i * NB_LAST
        pl.when(b0 % NB_MIDDLE == 0)(
            lambda: _wait(kv_copies(NPAIR - 1, b0, NB_MIDDLE, NB_MIDDLE)))
        compute(NPAIR - 1, b0, NB_LAST, "last")

    _start(w_copies(0))
    for b in range(2):
        _start(x_copies(b) + kv_copies(0, b, 1, 1))
    probe[...] = jnp.zeros_like(probe)
    _wait(w_copies(0))
    for b in range(2, AHEAD):
        _start(x_copies(b) + kv_copies(0, b, 1, 1))
    lax.fori_loop(0, B, first_step, None)

    for b in range(AHEAD, B, NB_SECOND):
        _start(kv_copies(1, b, NB_SECOND, NB_SECOND))
    middle_pair(1, NB_SECOND)
    lax.fori_loop(2, NPAIR - 1, lambda g, _: middle_pair(g, NB_MIDDLE), None)

    _wait(w_copies(NPAIR - 1))
    lax.fori_loop(0, B // NB_LAST, last_step, None)
    saw_nan = jnp.sum(jnp.where(probe[...] == probe[...], 0.0, 1.0)) > 0.0
    _wait([out_copy(b) for b in range(B)])

    @pl.when(saw_nan)
    def _recompute_with_plain_scores():
        def clear(b, _):
            _start(kv_copies(0, b, 1, 1))
            acc[b] = jnp.zeros((SQ, 2 * D), f32)

        def pair(g, _):
            _wait(w_copies(g))
            pl.when(g + 1 < NPAIR)(lambda: _start(w_copies(g + 1)))

            def step(b, _):
                _wait(kv_copies(g, b, 1, 1))
                compute(g, b, 1, "middle", plain=True)
                pl.when(g + 1 < NPAIR)(lambda: _start(kv_copies(g + 1, b, 1, 1)))

            lax.fori_loop(0, B, step, None)

        def store(b, _):
            obuf[b] = acc[b].astype(bf16)
            out_copy(b).start()

        _start(w_copies(0))
        lax.fori_loop(0, B, clear, None)
        lax.fori_loop(0, NPAIR, pair, None)
        lax.fori_loop(0, B, store, None)
        _wait([out_copy(b) for b in range(B)])


@jax.jit
def pallas_concat_heads__gqa_block_cached__mha_block_cached__near_ridge_kernel(
    A_x: jax.Array,
    A_k_cache: jax.Array,
    A_v_cache: jax.Array,
    A_wq: jax.Array,
    A_wo: jax.Array,
    B_x: jax.Array,
    B_k_cache: jax.Array,
    B_v_cache: jax.Array,
    B_wq: jax.Array,
    B_wo: jax.Array,
):
    def features_by_keys(cache):
        return jnp.transpose(cache, (0, 1, 3, 2)).reshape(B, H * DH, SK)

    hbm = pl.BlockSpec(memory_space=pl.ANY)
    return pl.pallas_call(
        _kernel,
        in_specs=[hbm] * 10,
        out_specs=hbm,
        out_shape=jax.ShapeDtypeStruct((B, SQ, 2 * D), bf16),
        scratch_shapes=[
            pltpu.VMEM((2, B, SQ, D), bf16),
            pltpu.VMEM((2, B, PAIR, SK), bf16),
            pltpu.VMEM((2, B, PAIR, SK), bf16),
            pltpu.VMEM((2, 2, D, PAIR), bf16),
            pltpu.VMEM((2, 2, PAIR, D), bf16),
            pltpu.VMEM((B, SQ, 2 * D), f32),
            pltpu.VMEM((B, SQ, 2 * D), bf16),
            pltpu.VMEM((8, 128), f32),
            pltpu.SemaphoreType.DMA((B,)),
            pltpu.SemaphoreType.DMA((2,)),
            pltpu.SemaphoreType.DMA(()),
        ],
        compiler_params=pltpu.CompilerParams(vmem_limit_bytes=100 * 1024 * 1024),
    )(A_x, features_by_keys(A_k_cache), features_by_keys(A_v_cache), A_wq, A_wo,
      B_x, features_by_keys(B_k_cache), features_by_keys(B_v_cache), B_wq, B_wo)
```
